```python
import os as _os
_os.environ.setdefault("JAX_PLATFORMS", "cpu")
import jax
import jax.numpy as jnp

def _softmax(x, axis=-1):
    return jax.nn.softmax(x, axis=axis)
def _gelu(x):
    return jax.nn.gelu(x, approximate=True)
def _silu(x):
    return jax.nn.silu(x)
def _sigmoid(x):
    return jax.nn.sigmoid(x)
def _layernorm(x, axis=-1, eps=1e-5):
    m = jnp.mean(x, axis=axis, keepdims=True)
    v = jnp.var(x, axis=axis, keepdims=True)
    return (x - m) / jnp.sqrt(v + eps)
def _scatter_add(tgt, idx, src, axis=0):
    return tgt.at[idx].add(src)
def _segment_sum(src, seg, n):
    return jax.ops.segment_sum(src, seg, n)
class _Rng:
    def __init__(self, key):
        self._k = key
    def _next(self):
        self._k, sub = jax.random.split(self._k)
        return sub
    def normal(self, shape):
        return jax.random.normal(self._next(), shape, dtype=jnp.bfloat16)
    def randint(self, lo, hi, shape):
        return jax.random.randint(self._next(), shape, lo, hi, dtype=jnp.int32)
    def uniform(self, shape, lo=0.0, hi=1.0):
        return jax.random.uniform(self._next(), shape, jnp.bfloat16, lo, hi)
    def permutation(self, n):
        return jax.random.permutation(self._next(), n)


kernel_name = 'standalone__gqa_block_cached__near_ridge'

def setup_inputs():
    _rng = _Rng(jax.random.key(int.from_bytes(__import__("os").urandom(4), "little")))
    _w = (lambda a: (lambda t: t.astype(jnp.bfloat16) if jnp.issubdtype(t.dtype, jnp.floating) else t)(jnp.asarray(a)))
    B, Sq, D = 8, 96, 448
    Hq, Hkv, Sk, Dh = 16, 8, 2048, 256
    assert Hq % Hkv == 0, (Hq, Hkv)
    return {
        "x": _w((lambda *s: _rng.normal(s) * 0.8)(B, Sq, D)),
        "k_cache": _w((lambda *s: _rng.normal(s) * 0.8)(B, Hkv, Sk, Dh)),
        "v_cache": _w((lambda *s: _rng.normal(s) * 0.05)(B, Hkv, Sk, Dh)),
        "wq": _w((lambda *s: _rng.normal(s) * 0.8)(D, Hq * Dh) * (D ** -0.5)),
        "wo": _w((lambda *s: _rng.normal(s) * 0.05)(Hq * Dh, D) * ((Hq * Dh) ** -0.5)),
    }

def reference(x, k_cache, v_cache, wq, wo):
    B, Sq, D = x.shape
    Hq, Dh = 16, 256
    Hkv = k_cache.shape[1]
    rep = Hq // Hkv
    q = (lambda x, *d: x.transpose(*d))((x @ wq).reshape(B, Sq, Hq, Dh), 0, 2, 1, 3)
    k = jnp.repeat(k_cache, rep, axis=1)
    v = jnp.repeat(v_cache, rep, axis=1)
    scores = jnp.einsum("bhqd,bhkd->bhqk", q, k) * (Dh ** -0.5)
    p = _softmax(scores, axis=-1)
    o = jnp.einsum("bhqk,bhkd->bhqd", p, v)
    return (lambda x, *d: x.transpose(*d))(o, 0, 2, 1, 3).reshape(B, Sq, Hq * Dh) @ wo
```

```python
import functools
import math
import jax
import jax.numpy as jnp
import jax.experimental.pallas as pl
import jax.experimental.pallas.tpu as pltpu

NBUF = 4
NC = 2

_NT = (((1,), (1,)), ((), ()))


def _kernel(x_hbm, k_hbm, v_hbm, wq_hbm, wot_hbm, out_hbm,
            x_v, wq_v, wot_v, kbuf, vbuf, q_sc, o_sc, acc_sc, out_v,
            ksem, vsem, wqsem, wosem, xsem, osem,
            *, B, Sq, Hkv, Sk, Dh, rep, qscale):
    nsteps = Hkv * B
    HW = rep * Dh

    def k_copy(step, slot):
        return pltpu.make_async_copy(k_hbm.at[step % B, step // B], kbuf.at[slot], ksem.at[slot])

    def v_copy(step, slot):
        return pltpu.make_async_copy(v_hbm.at[step % B, step // B], vbuf.at[slot], vsem.at[slot])

    def wq_copy(h, slot):
        return pltpu.make_async_copy(wq_hbm.at[:, pl.ds(pl.multiple_of(h * HW, HW), HW)], wq_v.at[slot], wqsem.at[slot])

    def wo_copy(h, slot):
        return pltpu.make_async_copy(wot_hbm.at[:, pl.ds(pl.multiple_of(h * HW, HW), HW)], wot_v.at[slot], wosem.at[slot])

    x_copy = pltpu.make_async_copy(x_hbm, x_v, xsem.at[0])

    x_copy.start()
    wq_copy(0, 0).start()
    for j in range(NBUF - 1):
        k_copy(j, j).start()
        v_copy(j, j).start()
    wo_copy(0, 0).start()
    acc_sc[...] = jnp.zeros_like(acc_sc)
    x_copy.wait()

    def attention(slot, q2):
        CK = Sk // NC
        ms, ls, os_ = [], [], []
        for c in range(NC):
            kc = kbuf[slot, pl.ds(c * CK, CK), :]
            s = jax.lax.dot_general(q2, kc, _NT, preferred_element_type=jnp.float32)
            m = jnp.max(s, axis=-1, keepdims=True)
            p = jnp.exp2(s - m)
            l = jnp.sum(p, axis=-1, keepdims=True)
            vc = vbuf[slot, pl.ds(c * CK, CK), :]
            o = jnp.dot(p.astype(vc.dtype), vc, preferred_element_type=jnp.float32)
            ms.append(m); ls.append(l); os_.append(o)
        m = functools.reduce(jnp.maximum, ms)
        al = [jnp.exp2(mc - m) for mc in ms]
        l = functools.reduce(jnp.add, [a * lc for a, lc in zip(al, ls)])
        inv = 1.0 / l
        return functools.reduce(jnp.add, [(a * inv) * oc for a, oc in zip(al, os_)])

    def head_body(h, carry):
        hs = h % 2
        wq_copy(h, hs).wait()

        @pl.when(h + 1 < Hkv)
        def _():
            wq_copy(h + 1, 1 - hs).start()

        q = jnp.dot(x_v[...], wq_v[hs], preferred_element_type=jnp.float32)
        q = (q * qscale).astype(q_sc.dtype)
        for b in range(B):
            for r in range(rep):
                q_sc[b, r * Sq:(r + 1) * Sq, :] = q[b * Sq:(b + 1) * Sq, r * Dh:(r + 1) * Dh]

        def batch_body(b, carry2):
            step = h * B + b
            slot = step % NBUF
            nxt = step + NBUF - 1

            @pl.when(nxt < nsteps)
            def _():
                k_copy(nxt, nxt % NBUF).start()
                v_copy(nxt, nxt % NBUF).start()

            k_copy(step, slot).wait()
            v_copy(step, slot).wait()
            o = attention(slot, q_sc[b])
            row = pl.multiple_of(b * Sq, 16)
            for r in range(rep):
                o_sc[pl.ds(row, Sq), r * Dh:(r + 1) * Dh] = o[r * Sq:(r + 1) * Sq, :].astype(o_sc.dtype)
            return carry2

        jax.lax.fori_loop(0, B, batch_body, 0)

        wo_copy(h, hs).wait()

        @pl.when(h + 1 < Hkv)
        def _():
            wo_copy(h + 1, 1 - hs).start()

        acc_sc[...] += jax.lax.dot_general(o_sc[...], wot_v[hs], _NT, preferred_element_type=jnp.float32)
        return carry

    jax.lax.fori_loop(0, Hkv, head_body, 0)
    out_v[...] = acc_sc[...].astype(out_v.dtype)
    oc = pltpu.make_async_copy(out_v, out_hbm, osem.at[0])
    oc.start()
    oc.wait()


@jax.jit
def pallas_standalone__gqa_block_cached__near_ridge_kernel(x, k_cache, v_cache, wq, wo):
    B, Sq, D = x.shape
    _, Hkv, Sk, Dh = k_cache.shape
    Hq = wq.shape[1] // Dh
    rep = Hq // Hkv
    qscale = (Dh ** -0.5) * math.log2(math.e)
    x2 = x.reshape(B * Sq, D)
    wot = wo.T
    kern = functools.partial(_kernel, B=B, Sq=Sq, Hkv=Hkv, Sk=Sk, Dh=Dh, rep=rep, qscale=qscale)
    bf = jnp.bfloat16
    out = pl.pallas_call(
        kern,
        in_specs=[pl.BlockSpec(memory_space=pl.ANY)] * 5,
        out_specs=pl.BlockSpec(memory_space=pl.ANY),
        out_shape=jax.ShapeDtypeStruct((B * Sq, D), x.dtype),
        scratch_shapes=[
            pltpu.VMEM((B * Sq, D), bf),
            pltpu.VMEM((2, D, rep * Dh), bf),
            pltpu.VMEM((2, D, rep * Dh), bf),
            pltpu.VMEM((NBUF, Sk, Dh), bf),
            pltpu.VMEM((NBUF, Sk, Dh), bf),
            pltpu.VMEM((B, rep * Sq, Dh), bf),
            pltpu.VMEM((B * Sq, rep * Dh), bf),
            pltpu.VMEM((B * Sq, D), jnp.float32),
            pltpu.VMEM((B * Sq, D), x.dtype),
            pltpu.SemaphoreType.DMA((NBUF,)),
            pltpu.SemaphoreType.DMA((NBUF,)),
            pltpu.SemaphoreType.DMA((2,)),
            pltpu.SemaphoreType.DMA((2,)),
            pltpu.SemaphoreType.DMA((1,)),
            pltpu.SemaphoreType.DMA((1,)),
        ],
        compiler_params=pltpu.CompilerParams(
            vmem_limit_bytes=64 * 1024 * 1024,
        ),
    )(x2, k_cache, v_cache, wq, wot)
    return out.reshape(B, Sq, D)
```

```python
import functools
import math
import jax
import jax.numpy as jnp
import jax.experimental.pallas as pl
import jax.experimental.pallas.tpu as pltpu

NBUF = 4
NC = 4
NBANK = 1

_NT = (((1,), (1,)), ((), ()))


def _kernel(x_hbm, k_hbm, v_hbm, wq_hbm, wot_hbm, out_hbm,
            x_v, wq_v, wot_v, kbuf, vbuf, q_bank, acc_sc, out_v,
            ksem, vsem, wqsem, wosem, xsem, osem, v2sem,
            *, B, Sq, Hkv, Sk, Dh, rep, qscale):
    nsteps = Hkv * B
    last = nsteps - 1
    HW = rep * Dh
    CK = Sk // NC
    H1 = Hkv - NBANK
    S2 = H1 * B
    HALF = Sk // 2
    div = jax.lax.div
    rem = jax.lax.rem
    i32 = jnp.int32
    bf16 = jnp.bfloat16

    def k_copy(step, slot):
        return pltpu.make_async_copy(k_hbm.at[rem(step, B), div(step, B)], kbuf.at[slot], ksem.at[slot])

    def v_copy(step, slot):
        return pltpu.make_async_copy(v_hbm.at[rem(step, B), div(step, B)], vbuf.at[slot], vsem.at[slot])

    def v_half_copy(part):
        lslot = last % NBUF
        return pltpu.make_async_copy(
            v_hbm.at[B - 1, Hkv - 1, pl.ds(part * HALF, HALF)],
            vbuf.at[lslot, pl.ds(part * HALF, HALF)], v2sem.at[part])

    def wq_copy(h, slot):
        return pltpu.make_async_copy(wq_hbm.at[:, pl.ds(pl.multiple_of(h * HW, HW), HW)], wq_v.at[slot], wqsem.at[slot])

    def wo_copy(h, slot):
        return pltpu.make_async_copy(wot_hbm.at[:, pl.ds(pl.multiple_of(h * HW, HW), HW)], wot_v.at[slot], wosem.at[slot])

    def out_copy(b0, nb, s):
        return pltpu.make_async_copy(out_v.at[pl.ds(b0, nb)], out_hbm.at[pl.ds(b0, nb)], osem.at[s])

    x_copy = pltpu.make_async_copy(x_hbm, x_v, xsem.at[0])
    groups = [lambda: (x_copy.start(), wq_copy(i32(0), 0).start())]
    groups += [functools.partial(lambda j: wq_copy(i32(H1 + j), 2 + j).start(), j) for j in range(NBANK)]
    groups += [lambda: k_copy(i32(0), 0).start(), lambda: v_copy(i32(0), 0).start(),
               lambda: wo_copy(i32(0), 0).start()]
    for j in range(1, NBUF - 1):
        groups += [functools.partial(lambda j: k_copy(i32(j), j).start(), j),
                   functools.partial(lambda j: v_copy(i32(j), j).start(), j)]

    def issue(j, c):
        for g, fn in enumerate(groups):
            pl.when(j == g)(lambda fn=fn: (fn(), None)[1])
        return c

    jax.lax.fori_loop(0, len(groups), issue, 0)
    acc_sc[...] = jnp.zeros_like(acc_sc)

    def qproj(b, hslot):
        q = jnp.dot(x_v[b], wq_v[hslot], preferred_element_type=jnp.float32)
        q = (q * qscale).astype(bf16)
        return jnp.concatenate([q[:, r * Dh:(r + 1) * Dh] for r in range(rep)], axis=0)

    def oproj(b, hslot, o2):
        new = acc_sc[b] + jax.lax.dot_general(o2, wot_v[hslot], _NT, preferred_element_type=jnp.float32)
        acc_sc[b] = new
        out_v[b] = new.astype(out_v.dtype)

    def qk(slot, q2, c):
        kc = kbuf[slot, pl.ds(c * CK, CK), :]
        s = jax.lax.dot_general(q2, kc, _NT, preferred_element_type=jnp.float32)
        m = jnp.max(s, axis=-1, keepdims=True)
        p = jnp.exp2(s - m)
        l = jnp.sum(p, axis=-1, keepdims=True)
        return m, l, p.astype(bf16)

    def pv(slot, p, c):
        vc = vbuf[slot, pl.ds(c * CK, CK), :]
        return jnp.dot(p, vc, preferred_element_type=jnp.float32)

    def combine(ms, ls, os_):
        m = functools.reduce(jnp.maximum, ms)
        al = [jnp.exp2(mc - m) for mc in ms]
        l = functools.reduce(jnp.add, [a * lc for a, lc in zip(al, ls)])
        inv = 1.0 / l
        o = functools.reduce(jnp.add, [(a * inv) * oc for a, oc in zip(al, os_)])
        o = o.astype(bf16)
        return jnp.concatenate([o[r * Sq:(r + 1) * Sq, :] for r in range(rep)], axis=1)

    def attention_coarse(slot, q2, filler):
        st = [qk(slot, q2, 0)]
        os_ = []
        for c in range(1, NC):
            st.append(qk(slot, q2, c))
            os_.append(pv(slot, st[c - 1][2], c - 1))
        filler()
        os_.append(pv(slot, st[NC - 1][2], NC - 1))
        return combine([t[0] for t in st], [t[1] for t in st], os_)

    def prefetch_k_and_weights(i):
        h = div(i, B)
        b = rem(i, B)
        nxt = i + (NBUF - 1)

        @pl.when(nxt <= last)
        def _():
            k_copy(nxt, rem(nxt, NBUF)).start()

        @pl.when(jnp.logical_and(b == 1, h > 0))
        def _():
            wo_copy(h, rem(h, 2)).wait()

        return h, b

    def prefetch_v(i):
        nxt = i + (NBUF - 1)

        @pl.when(nxt < last)
        def _():
            v_copy(nxt, rem(nxt, NBUF)).start()

        @pl.when(nxt == last)
        def _():
            v_half_copy(0).start()

    def prefetch_rest(i):
        h = div(i, B)
        b = rem(i, B)
        nxt = i + (NBUF - 1)

        @pl.when(nxt == last)
        def _():
            v_half_copy(1).start()

        @pl.when(jnp.logical_and(b == 2, h + 1 < Hkv))
        def _():
            wo_copy(h + 1, rem(h + 1, 2)).start()

        @pl.when(jnp.logical_and(b == 0, h + 1 < H1))
        def _():
            wq_copy(h + 1, rem(h + 1, 2)).start()

    x_copy.wait()
    wq_copy(i32(0), 0).wait()
    q0 = qproj(0, 0)
    xall = x_v[...].reshape(B * Sq, x_v.shape[-1])
    for j in range(NBANK):
        wq_copy(i32(H1 + j), 2 + j).wait()
        q = jnp.dot(xall, wq_v[2 + j], preferred_element_type=jnp.float32)
        q = (q * qscale).astype(bf16)
        for b in range(B):
            for r in range(rep):
                q_bank[j * B + b, r * Sq:(r + 1) * Sq, :] = q[b * Sq:(b + 1) * Sq, r * Dh:(r + 1) * Dh]
    wo_copy(i32(0), 0).wait()

    def body1(i, carry):
        q_cur, o_prev = carry
        h, b = prefetch_k_and_weights(i)
        slot = rem(i, NBUF)

        @pl.when(jnp.logical_and(b == B - 1, h + 1 < H1))
        def _():
            wq_copy(h + 1, rem(h + 1, 2)).wait()

        k_copy(i, slot).wait()
        prefetch_v(i)
        v_copy(i, slot).wait()
        prefetch_rest(i)

        ip = jnp.maximum(i - 1, 0)
        inx = i + 1
        hn = div(inx, B)
        o2 = attention_coarse(slot, q_cur, lambda: oproj(rem(ip, B), rem(div(ip, B), 2), o_prev))
        q_next = qproj(rem(inx, B), jnp.where(hn < H1, rem(hn, 2), 2))
        return q_next, o2

    o_init = jnp.zeros((Sq, HW), bf16)
    _, o_prev = jax.lax.fori_loop(0, S2, body1, (q0, o_init))

    def body2(i, o_prev):
        prefetch_k_and_weights(i)
        slot = rem(i, NBUF)
        ip = i - 1
        k_copy(i, slot).wait()
        prefetch_v(i)
        q2 = q_bank[i - S2]
        st = [qk(slot, q2, c) for c in range(NC)]
        oproj(rem(ip, B), rem(div(ip, B), 2), o_prev)
        v_copy(i, slot).wait()
        prefetch_rest(i)
        os_ = [pv(slot, st[c][2], c) for c in range(NC)]
        return combine([t[0] for t in st], [t[1] for t in st], os_)

    o_prev = jax.lax.fori_loop(S2, last, body2, o_prev)

    lslot = last % NBUF
    hs = (Hkv - 1) % 2
    out_copy(0, B - 2, 0).start()
    k_copy(i32(last), lslot).wait()
    q2 = q_bank[last - S2]
    st = [qk(lslot, q2, c) for c in range(NC)]
    v_half_copy(0).wait()
    os_ = [pv(lslot, st[c][2], c) for c in range(NC // 2)]
    oproj(B - 2, hs, o_prev)
    v_half_copy(1).wait()
    out_copy(B - 2, 1, 1).start()
    os_ += [pv(lslot, st[c][2], c) for c in range(NC // 2, NC)]
    o2 = combine([t[0] for t in st], [t[1] for t in st], os_)
    oproj(B - 1, hs, o2)
    out_copy(B - 1, 1, 2).start()
    out_copy(0, B - 2, 0).wait()
    out_copy(B - 2, 1, 1).wait()
    out_copy(B - 1, 1, 2).wait()


@jax.jit
def pallas_standalone__gqa_block_cached__near_ridge_kernel(x, k_cache, v_cache, wq, wo):
    B, Sq, D = x.shape
    _, Hkv, Sk, Dh = k_cache.shape
    Hq = wq.shape[1] // Dh
    rep = Hq // Hkv
    qscale = (Dh ** -0.5) * math.log2(math.e)
    wot = wo.T
    kern = functools.partial(_kernel, B=B, Sq=Sq, Hkv=Hkv, Sk=Sk, Dh=Dh, rep=rep, qscale=qscale)
    bf = jnp.bfloat16
    return pl.pallas_call(
        kern,
        in_specs=[pl.BlockSpec(memory_space=pl.ANY)] * 5,
        out_specs=pl.BlockSpec(memory_space=pl.ANY),
        out_shape=jax.ShapeDtypeStruct((B, Sq, D), x.dtype),
        scratch_shapes=[
            pltpu.VMEM((B, Sq, D), bf),
            pltpu.VMEM((2 + NBANK, D, rep * Dh), bf),
            pltpu.VMEM((2, D, rep * Dh), bf),
            pltpu.VMEM((NBUF, Sk, Dh), bf),
            pltpu.VMEM((NBUF, Sk, Dh), bf),
            pltpu.VMEM((NBANK * B, rep * Sq, Dh), bf),
            pltpu.VMEM((B, Sq, D), jnp.float32),
            pltpu.VMEM((B, Sq, D), x.dtype),
            pltpu.SemaphoreType.DMA((NBUF,)),
            pltpu.SemaphoreType.DMA((NBUF,)),
            pltpu.SemaphoreType.DMA((2 + NBANK,)),
            pltpu.SemaphoreType.DMA((2,)),
            pltpu.SemaphoreType.DMA((1,)),
            pltpu.SemaphoreType.DMA((3,)),
            pltpu.SemaphoreType.DMA((2,)),
        ],
        compiler_params=pltpu.CompilerParams(
            vmem_limit_bytes=64 * 1024 * 1024,
            disable_bounds_checks=True,
        ),
    )(x, k_cache, v_cache, wq, wot)
```

```python
import functools
import math

import jax
import jax.numpy as jnp
import jax.experimental.pallas as pl
import jax.experimental.pallas.tpu as pltpu

NBUF = 4
NC = 4
NBANK = 2

_NT = (((1,), (1,)), ((), ()))


def _kernel(x_hbm, k_hbm, v_hbm, wq_hbm, wot_hbm, out_hbm,
            x_v, wq_v, wot_v, kbuf, vbuf, q_bank, acc_sc, out_v,
            ksem, vsem, wqsem, wosem, xsem, osem,
            *, B, Sq, Hkv, Sk, Dh, rep, qscale):
    nsteps = Hkv * B
    last = nsteps - 1
    HW = rep * Dh
    CK = Sk // NC
    H1 = Hkv - NBANK
    S2 = H1 * B
    div = jax.lax.div
    rem = jax.lax.rem
    i32 = jnp.int32
    bf16 = jnp.bfloat16

    def k_copy(step, slot):
        return pltpu.make_async_copy(k_hbm.at[rem(step, B), div(step, B)], kbuf.at[slot], ksem.at[slot])

    def v_copy(step, slot):
        return pltpu.make_async_copy(v_hbm.at[rem(step, B), div(step, B)], vbuf.at[slot], vsem.at[slot])

    def wq_copy(h, slot):
        cols = pl.ds(pl.multiple_of(h * HW, HW), HW)
        return pltpu.make_async_copy(wq_hbm.at[:, cols], wq_v.at[slot], wqsem.at[slot])

    def wo_copy(h, slot):
        cols = pl.ds(pl.multiple_of(h * HW, HW), HW)
        return pltpu.make_async_copy(wot_hbm.at[:, cols], wot_v.at[slot], wosem.at[slot])

    def out_copy(b0, nb, s):
        return pltpu.make_async_copy(out_v.at[pl.ds(b0, nb)], out_hbm.at[pl.ds(b0, nb)], osem.at[s])

    x_copy = pltpu.make_async_copy(x_hbm, x_v, xsem.at[0])

    groups = [[x_copy, wq_copy(i32(0), 0)]]
    groups += [[wq_copy(i32(H1 + j), 2 + j)] for j in range(NBANK)]
    groups += [[k_copy(i32(0), 0)], [v_copy(i32(0), 0)], [wo_copy(i32(0), 0)]]
    for j in range(1, NBUF - 1):
        groups += [[k_copy(i32(j), j)], [v_copy(i32(j), j)]]

    def issue(j, c):
        for g, copies in enumerate(groups):
            @pl.when(j == g)
            def _(copies=copies):
                for cp in copies:
                    cp.start()
        return c

    jax.lax.fori_loop(0, len(groups), issue, 0)
    acc_sc[...] = jnp.zeros_like(acc_sc)

    def qproj(b, hslot):
        q = jnp.dot(x_v[b], wq_v[hslot], preferred_element_type=jnp.float32)
        q = (q * qscale).astype(bf16)
        return jnp.concatenate([q[:, r * Dh:(r + 1) * Dh] for r in range(rep)], axis=0)

    def oproj(b, hslot, o2):
        new = acc_sc[b] + jax.lax.dot_general(o2, wot_v[hslot], _NT, preferred_element_type=jnp.float32)
        acc_sc[b] = new
        out_v[b] = new.astype(out_v.dtype)

    def qk(slot, q2, c):
        kc = kbuf[slot, pl.ds(c * CK, CK), :]
        s = jax.lax.dot_general(q2, kc, _NT, preferred_element_type=jnp.float32)
        m = jnp.max(s, axis=-1, keepdims=True)
        p = jnp.exp2(s - m)
        l = jnp.sum(p, axis=-1, keepdims=True)
        return m, l, p.astype(bf16)

    def pv(slot, p, c):
        vc = vbuf[slot, pl.ds(c * CK, CK), :]
        return jnp.dot(p, vc, preferred_element_type=jnp.float32)

    def combine(st, os_):
        ms = [t[0] for t in st]
        m = functools.reduce(jnp.maximum, ms)
        al = [jnp.exp2(mc - m) for mc in ms]
        l = functools.reduce(jnp.add, [a * t[1] for a, t in zip(al, st)])
        inv = 1.0 / l
        o = functools.reduce(jnp.add, [(a * inv) * oc for a, oc in zip(al, os_)])
        o = o.astype(bf16)
        return jnp.concatenate([o[r * Sq:(r + 1) * Sq, :] for r in range(rep)], axis=1)

    def prefetch_k(i):
        nxt = i + (NBUF - 1)

        @pl.when(nxt <= last)
        def _():
            k_copy(nxt, rem(nxt, NBUF)).start()

        @pl.when(jnp.logical_and(rem(i, B) == 1, i >= B))
        def _():
            h = div(i, B)
            wo_copy(h, rem(h, 2)).wait()

    def prefetch_v(i):
        nxt = i + (NBUF - 1)

        @pl.when(nxt <= last)
        def _():
            v_copy(nxt, rem(nxt, NBUF)).start()

    def prefetch_weights(i):
        h = div(i, B)
        b = rem(i, B)

        @pl.when(jnp.logical_and(b == 2, h + 1 < Hkv))
        def _():
            wo_copy(h + 1, rem(h + 1, 2)).start()

        @pl.when(jnp.logical_and(b == 0, h + 1 < H1))
        def _():
            wq_copy(h + 1, rem(h + 1, 2)).start()

    x_copy.wait()
    wq_copy(i32(0), 0).wait()
    q0 = qproj(0, 0)
    for j in range(NBANK):
        wq_copy(i32(H1 + j), 2 + j).wait()
        for b in range(B):
            q_bank[j * B + b] = qproj(b, 2 + j)
    wo_copy(i32(0), 0).wait()

    def body1(i, carry):
        q_cur, o_prev = carry
        slot = rem(i, NBUF)
        prefetch_k(i)
        inx = i + 1
        hn = div(inx, B)

        @pl.when(jnp.logical_and(rem(inx, B) == 0, hn < H1))
        def _():
            wq_copy(hn, rem(hn, 2)).wait()

        k_copy(i, slot).wait()
        prefetch_v(i)
        v_copy(i, slot).wait()
        prefetch_weights(i)

        ip = jnp.maximum(i - 1, 0)
        st = [qk(slot, q_cur, 0)]
        os_ = []
        for c in range(1, NC):
            st.append(qk(slot, q_cur, c))
            os_.append(pv(slot, st[c - 1][2], c - 1))
        oproj(rem(ip, B), rem(div(ip, B), 2), o_prev)
        os_.append(pv(slot, st[NC - 1][2], NC - 1))
        o2 = combine(st, os_)
        q_next = qproj(rem(inx, B), jnp.where(hn < H1, rem(hn, 2), 2))
        return q_next, o2

    _, o_prev = jax.lax.fori_loop(0, S2, body1, (q0, jnp.zeros((Sq, HW), bf16)))

    def body2(i, o_prev):
        slot = rem(i, NBUF)
        ip = i - 1
        prefetch_k(i)
        k_copy(i, slot).wait()
        prefetch_v(i)
        q2 = q_bank[i - S2]
        st = [qk(slot, q2, c) for c in range(NC)]
        oproj(rem(ip, B), rem(div(ip, B), 2), o_prev)
        v_copy(i, slot).wait()
        prefetch_weights(i)
        return combine(st, [pv(slot, st[c][2], c) for c in range(NC)])

    o_prev = jax.lax.fori_loop(S2, last, body2, o_prev)

    lslot = last % NBUF
    hs = (Hkv - 1) % 2
    k_copy(i32(last), lslot).wait()
    q2 = q_bank[last - S2]
    st = [qk(lslot, q2, c) for c in range(NC)]
    oproj(B - 2, hs, o_prev)
    v_copy(i32(last), lslot).wait()
    out_copy(0, B - 1, 0).start()
    o2 = combine(st, [pv(lslot, st[c][2], c) for c in range(NC)])
    oproj(B - 1, hs, o2)
    out_copy(B - 1, 1, 1).start()
    out_copy(0, B - 1, 0).wait()
    out_copy(B - 1, 1, 1).wait()


@jax.jit
def pallas_standalone__gqa_block_cached__near_ridge_kernel(
    x: jax.Array,
    k_cache: jax.Array,
    v_cache: jax.Array,
    wq: jax.Array,
    wo: jax.Array,
):
    B, Sq, D = x.shape
    _, Hkv, Sk, Dh = k_cache.shape
    Hq = wq.shape[1] // Dh
    rep = Hq // Hkv
    qscale = (Dh ** -0.5) * math.log2(math.e)
    wot = wo.T
    kern = functools.partial(_kernel, B=B, Sq=Sq, Hkv=Hkv, Sk=Sk, Dh=Dh, rep=rep, qscale=qscale)
    bf = jnp.bfloat16
    return pl.pallas_call(
        kern,
        in_specs=[pl.BlockSpec(memory_space=pl.ANY)] * 5,
        out_specs=pl.BlockSpec(memory_space=pl.ANY),
        out_shape=jax.ShapeDtypeStruct((B, Sq, D), x.dtype),
        scratch_shapes=[
            pltpu.VMEM((B, Sq, D), x.dtype),
            pltpu.VMEM((2 + NBANK, D, rep * Dh), wq.dtype),
            pltpu.VMEM((2, D, rep * Dh), wo.dtype),
            pltpu.VMEM((NBUF, Sk, Dh), k_cache.dtype),
            pltpu.VMEM((NBUF, Sk, Dh), v_cache.dtype),
            pltpu.VMEM((NBANK * B, rep * Sq, Dh), bf),
            pltpu.VMEM((B, Sq, D), jnp.float32),
            pltpu.VMEM((B, Sq, D), x.dtype),
            pltpu.SemaphoreType.DMA((NBUF,)),
            pltpu.SemaphoreType.DMA((NBUF,)),
            pltpu.SemaphoreType.DMA((2 + NBANK,)),
            pltpu.SemaphoreType.DMA((2,)),
            pltpu.SemaphoreType.DMA((1,)),
            pltpu.SemaphoreType.DMA((2,)),
        ],
        compiler_params=pltpu.CompilerParams(
            vmem_limit_bytes=64 * 1024 * 1024,
        ),
    )(x, k_cache, v_cache, wq, wot)
```
